```python
import jax
import jax.numpy as jnp

def _softmax(x, axis=-1):
    return jax.nn.softmax(x, axis=axis)

def _gelu(x):
    return jax.nn.gelu(x, approximate=True)

def _silu(x):
    return jax.nn.silu(x)

def _sigmoid(x):
    return jax.nn.sigmoid(x)

def _layernorm(x, axis=-1, eps=1e-05):
    m = jnp.mean(x, axis=axis, keepdims=True)
    v = jnp.var(x, axis=axis, keepdims=True)
    return (x - m) / jnp.sqrt(v + eps)

def _scatter_add(tgt, idx, src, axis=0):
    return tgt.at[idx].add(src)

def _segment_sum(src, seg, n):
    return jax.ops.segment_sum(src, seg, n)

class _Rng:

    def __init__(self, key):
        self._k = key

    def _next(self):
        self._k, sub = jax.random.split(self._k)
        return sub

    def normal(self, shape):
        return jax.random.normal(self._next(), shape, dtype=jnp.bfloat16)

    def randint(self, lo, hi, shape):
        return jax.random.randint(self._next(), shape, lo, hi, dtype=jnp.int32)

    def uniform(self, shape, lo=0.0, hi=1.0):
        return jax.random.uniform(self._next(), shape, jnp.bfloat16, lo, hi)

    def permutation(self, n):
        return jax.random.permutation(self._next(), n)
kernel_name = 'adaLN_cond__sliding_block_cached__moe_arch_mod__decode'

def setup_inputs():
    _rng = _Rng(jax.random.key(int.from_bytes(__import__("os").urandom(4), "little")))
    _w = lambda a: (lambda t: t.astype(jnp.bfloat16) if jnp.issubdtype(t.dtype, jnp.floating) else t)(jnp.asarray(a))

    def _A_setup():
        B, Sq, D = (8, 1, 576)
        Hq, Hkv, Sk, Dh = (32, 16, 8192, 128)
        assert Hq % Hkv == 0, (Hq, Hkv)
        return {'x': _w((lambda *s: _rng.normal(s) * 0.05)(B, Sq, D)), 'k_cache': _w((lambda *s: _rng.normal(s) * 0.05)(B, Hkv, Sk, Dh)), 'v_cache': _w((lambda *s: _rng.normal(s) * 0.05)(B, Hkv, Sk, Dh)), 'wq': _w((lambda *s: _rng.normal(s) * 0.05)(D, Hq * Dh) * D ** (-0.5)), 'wo': _w((lambda *s: _rng.normal(s) * 0.05)(Hq * Dh, D) * (Hq * Dh) ** (-0.5))}
    _A_in = _A_setup()

    def _B_setup():
        B, S, D, F, C = (8, 1, 576, 4608, 1)
        return {'x': _w((lambda *s: _rng.normal(s) * 0.05)(B, S, D)), 'w_r': _w((lambda *s: _rng.normal(s) * 0.05)(D)), 'w_gate': _w((lambda *s: _rng.normal(s) * 0.05)(D, F)), 'w_up': _w((lambda *s: _rng.normal(s) * 0.05)(D, F)), 'w_down': _w((lambda *s: _rng.normal(s) * 0.05)(F, D))}
    _B_in = _B_setup()
    return {'A_x': _A_in['x'], 'A_k_cache': _A_in['k_cache'], 'A_v_cache': _A_in['v_cache'], 'A_wq': _A_in['wq'], 'A_wo': _A_in['wo'], 'B_x': _B_in['x'], 'B_w_r': _B_in['w_r'], 'B_w_gate': _B_in['w_gate'], 'B_w_up': _B_in['w_up'], 'B_w_down': _B_in['w_down'], 'c': _w((lambda *s: _rng.normal(s) * 0.05)(8, 576)), 'w_mod': _w((lambda *s: _rng.normal(s) * 0.05)(576, 6 * 576) * 576 ** (-0.5))}

def reference(A_x, A_k_cache, A_v_cache, A_wq, A_wo, B_x, B_w_r, B_w_gate, B_w_up, B_w_down, c, w_mod):

    def _A_ref(x, k_cache, v_cache, wq, wo):
        B, Sq, D = x.shape
        Hq, Dh = (32, 128)
        Hkv, Sk = (k_cache.shape[1], k_cache.shape[2])
        W = min(4096, max(256, Sk // 4))
        rep = Hq // Hkv
        q = (lambda x, *d: x.transpose(*d))((x @ wq).reshape(B, Sq, Hq, Dh), 0, 2, 1, 3)
        k = jnp.repeat(k_cache[:, :, Sk - W:, :], rep, axis=1)
        v = jnp.repeat(v_cache[:, :, Sk - W:, :], rep, axis=1)
        scores = jnp.einsum('bhqd,bhkd->bhqk', q, k) * Dh ** (-0.5)
        p = _softmax(scores, axis=-1)
        o = jnp.einsum('bhqk,bhkd->bhqd', p, v)
        return (lambda x, *d: x.transpose(*d))(o, 0, 2, 1, 3).reshape(B, Sq, Hq * Dh) @ wo

    def _B_ref(x, w_r, w_gate, w_up, w_down):
        B, S, D = x.shape
        C = 1
        r = x @ w_r
        idx = jnp.argsort(-r, axis=-1)[:, :C]
        idx_e = jnp.repeat(idx.reshape(B, C, 1), D, axis=2)
        x_sel = jnp.take_along_axis(x, idx_e, axis=1)
        g = _silu(x_sel @ w_gate)
        u = x_sel @ w_up
        y = g * u @ w_down
        r_sel = _sigmoid(jnp.take_along_axis(r, idx, axis=1))
        y = y * r_sel.reshape(B, C, 1)
        b_off = (jnp.arange(B) * S).reshape(B, 1)
        flat_idx = (idx + b_off).reshape(B * C)
        zero = (x * 0.0).reshape(B * S, D)
        upd = _scatter_add(zero, flat_idx, y.reshape(B * C, D), axis=0)
        return x + upd.reshape(B, S, D)
    x = A_x
    mod = (_silu(c) @ w_mod).reshape(c.shape[0], 6, 1, -1)
    sa, ca, ga, sb, cb, gb = (mod[:, 0].copy(), mod[:, 1].copy(), mod[:, 2].copy(), mod[:, 3].copy(), mod[:, 4].copy(), mod[:, 5].copy())
    h = _layernorm(x, axis=-1) * (1 + ca) + sa
    x = x + ga * _A_ref(h, A_k_cache, A_v_cache, A_wq, A_wo)
    h = _layernorm(x, axis=-1) * (1 + cb) + sb
    x = x + gb * _B_ref(h, B_w_r, B_w_gate, B_w_up, B_w_down)
    return x
```

```python
import jax
import jax.numpy as jnp
from jax import lax
import jax.experimental.pallas as pl
import jax.experimental.pallas.tpu as pltpu

_NT = (((1,), (1,)), ((), ()))
_NN = (((1,), (0,)), ((), ()))
_F32 = jnp.float32
_BF16 = jnp.bfloat16


def _layernorm(x, eps=1e-05):
    m = jnp.mean(x, axis=-1, keepdims=True)
    xc = x - m
    v = jnp.mean(xc * xc, axis=-1, keepdims=True)
    return xc / jnp.sqrt(v + eps)


def _sigmoid(x):
    return 1.0 / (1.0 + jnp.exp(-x))


@jax.jit
def pallas_adaLN_cond__sliding_block_cached__moe_arch_mod__decode_kernel(
    A_x: jax.Array,
    A_k_cache: jax.Array,
    A_v_cache: jax.Array,
    A_wq: jax.Array,
    A_wo: jax.Array,
    B_x: jax.Array,
    B_w_r: jax.Array,
    B_w_gate: jax.Array,
    B_w_up: jax.Array,
    B_w_down: jax.Array,
    c: jax.Array,
    w_mod: jax.Array,
):
    B, Sq, D = A_x.shape
    _, Hkv, Sk, Dh = A_k_cache.shape
    Hq = A_wq.shape[1] // Dh
    F = B_w_gate.shape[1]
    W = min(4096, max(256, Sk // 4))
    rep = Hq // Hkv
    assert Sq == 1 and rep == 2 and B == 8
    scale = float(Dh) ** -0.5

    NSLOT = 3
    GU_CH = 4
    gu_w = F // GU_CH
    WD_SPLITS = (0, 1536, 3072, 4096, 4352, 4608)
    n_wd = len(WD_SPLITS) - 1
    MOD0 = 2 * D

    def kernel(x_hbm, k_hbm, v_hbm, wq_hbm, wot_hbm, wr_hbm, wg_hbm, wu_hbm,
               wdt_hbm, c_hbm, wmod_hbm, out_hbm,
               xbuf, cbuf, wrbuf, wmodbuf, wqbuf, wotbuf, wgbuf, wubuf, wdtbuf,
               kbuf, vbuf, qs, os_, obuf,
               misc_sems, kv_sems, gu_sems, wd_sems):
        cp_x = pltpu.make_async_copy(x_hbm, xbuf, misc_sems.at[0])
        cp_c = pltpu.make_async_copy(c_hbm, cbuf, misc_sems.at[1])
        cp_wr = pltpu.make_async_copy(wr_hbm, wrbuf, misc_sems.at[2])
        cp_mod0 = pltpu.make_async_copy(
            wmod_hbm.at[:, pl.ds(0, MOD0)], wmodbuf.at[:, pl.ds(0, MOD0)], misc_sems.at[3])
        cp_mod1 = pltpu.make_async_copy(
            wmod_hbm.at[:, pl.ds(MOD0, 6 * D - MOD0)],
            wmodbuf.at[:, pl.ds(MOD0, 6 * D - MOD0)], misc_sems.at[4])
        cp_wq = pltpu.make_async_copy(wq_hbm, wqbuf, misc_sems.at[5])
        cp_wo = pltpu.make_async_copy(wot_hbm, wotbuf, misc_sems.at[6])
        cp_out = pltpu.make_async_copy(obuf, out_hbm, misc_sems.at[7])

        def k_copy(h, slot):
            return pltpu.make_async_copy(
                k_hbm.at[:, h, pl.ds(Sk - W, W), :], kbuf.at[slot], kv_sems.at[0, slot])

        def v_copy(h, slot):
            return pltpu.make_async_copy(
                v_hbm.at[:, h, pl.ds(Sk - W, W), :], vbuf.at[slot], kv_sems.at[1, slot])

        def g_copy(j):
            sl = (slice(None), pl.ds(j * gu_w, gu_w))
            return pltpu.make_async_copy(wg_hbm.at[sl], wgbuf.at[sl], gu_sems.at[0, j])

        def u_copy(j):
            sl = (slice(None), pl.ds(j * gu_w, gu_w))
            return pltpu.make_async_copy(wu_hbm.at[sl], wubuf.at[sl], gu_sems.at[1, j])

        def d_copy(j):
            sl = (slice(None), pl.ds(WD_SPLITS[j], WD_SPLITS[j + 1] - WD_SPLITS[j]))
            return pltpu.make_async_copy(wdt_hbm.at[sl], wdtbuf.at[sl], wd_sems.at[j])

        cp_c.start()
        cp_x.start()
        cp_mod0.start()
        cp_wq.start()
        for s in range(NSLOT):
            k_copy(s, s).start()
            v_copy(s, s).start()
        cp_wr.start()

        cp_c.wait()
        cp_x.wait()
        cf = cbuf[...].astype(_F32)
        sc = (cf * _sigmoid(cf)).astype(_BF16)
        xf = xbuf[...].astype(_F32)
        xn = _layernorm(xf)
        cp_mod0.wait()
        mod0 = lax.dot_general(sc, wmodbuf[:, pl.ds(0, MOD0)], _NN,
                               preferred_element_type=_F32)
        h1 = (xn * (1.0 + mod0[:, D:2 * D]) + mod0[:, 0:D]).astype(_BF16)
        cp_wq.wait()
        q = lax.dot_general(h1, wqbuf[...], _NN, preferred_element_type=_F32)
        for h in range(Hkv):
            qs[h, 0:B, :] = q[:, (2 * h) * Dh:(2 * h + 1) * Dh]
            qs[h, B:2 * B, :] = q[:, (2 * h + 1) * Dh:(2 * h + 2) * Dh]

        row = lax.broadcasted_iota(jnp.int32, (2 * B, Dh), 0) % B

        def head_step(h, carry):
            slot = h % NSLOT
            q16 = qs[h]
            k_copy(h, slot).wait()
            s = None
            for b in range(B):
                qb = jnp.where(row == b, q16, 0.0).astype(_BF16)
                sb = lax.dot_general(qb, kbuf[slot, b], _NT, preferred_element_type=_F32)
                s = sb if s is None else s + sb
            s = s * scale
            m = jnp.max(s, axis=-1, keepdims=True)
            p = jnp.exp(s - m)
            l = jnp.sum(p, axis=-1, keepdims=True)
            pb = p.astype(_BF16)
            v_copy(h, slot).wait()
            o = jnp.zeros((2 * B, Dh), _F32)
            for b in range(B):
                ob = lax.dot_general(pb, vbuf[slot, b], _NN, preferred_element_type=_F32)
                o = jnp.where(row == b, ob, o)
            os_[h] = o / l

            @pl.when(h + NSLOT < Hkv)
            def _():
                k_copy(h + NSLOT, slot).start()
                v_copy(h + NSLOT, slot).start()

            @pl.when(h == 2)
            def _():
                cp_mod1.start()
                cp_wo.start()

            @pl.when(h + NSLOT == Hkv - 1)
            def _():
                for j in range(GU_CH):
                    g_copy(j).start()
                    u_copy(j).start()
                for j in range(n_wd):
                    d_copy(j).start()

            return carry

        lax.fori_loop(0, Hkv, head_step, 0)

        o_all = jnp.concatenate(
            [os_[h, pl.ds(r * B, B), :] for h in range(Hkv) for r in range(rep)],
            axis=1).astype(_BF16)
        cp_wo.wait()
        attn = lax.dot_general(o_all, wotbuf[...], _NT, preferred_element_type=_F32)
        cp_mod1.wait()
        mod1 = lax.dot_general(sc, wmodbuf[:, pl.ds(MOD0, 6 * D - MOD0)], _NN,
                               preferred_element_type=_F32)
        ga = mod1[:, 0:D]
        sb_ = mod1[:, D:2 * D]
        cb = mod1[:, 2 * D:3 * D]
        gb = mod1[:, 3 * D:4 * D]
        x1 = xf + ga * attn
        h2 = _layernorm(x1) * (1.0 + cb) + sb_
        h2b = h2.astype(_BF16)
        cp_wr.wait()
        wr = wrbuf[...].astype(_F32).reshape(1, D)
        r_sel = _sigmoid(jnp.sum(h2b.astype(_F32) * wr, axis=-1, keepdims=True))

        acts = []
        for j in range(GU_CH):
            g_copy(j).wait()
            g = lax.dot_general(h2b, wgbuf[:, pl.ds(j * gu_w, gu_w)], _NN,
                                preferred_element_type=_F32)
            u_copy(j).wait()
            u = lax.dot_general(h2b, wubuf[:, pl.ds(j * gu_w, gu_w)], _NN,
                                preferred_element_type=_F32)
            acts.append((g * _sigmoid(g) * u).astype(_BF16))
        act = jnp.concatenate(acts, axis=1)
        y = jnp.zeros((B, D), _F32)
        for j in range(n_wd):
            lo, hi = WD_SPLITS[j], WD_SPLITS[j + 1]
            d_copy(j).wait()
            y = y + lax.dot_general(act[:, lo:hi], wdtbuf[:, pl.ds(lo, hi - lo)], _NT,
                                    preferred_element_type=_F32)
        out = x1 + gb * (h2 + (h2 * 0.0 + y * r_sel))
        obuf[...] = out.astype(obuf.dtype)
        cp_out.start()
        cp_out.wait()

    any_spec = pl.BlockSpec(memory_space=pl.ANY)
    out = pl.pallas_call(
        kernel,
        out_shape=jax.ShapeDtypeStruct((B, D), A_x.dtype),
        in_specs=[any_spec] * 11,
        out_specs=any_spec,
        scratch_shapes=[
            pltpu.VMEM((B, D), _BF16),
            pltpu.VMEM((B, D), _BF16),
            pltpu.VMEM((D,), _BF16),
            pltpu.VMEM((D, 6 * D), _BF16),
            pltpu.VMEM((D, Hq * Dh), _BF16),
            pltpu.VMEM((D, Hq * Dh), _BF16),
            pltpu.VMEM((D, F), _BF16),
            pltpu.VMEM((D, F), _BF16),
            pltpu.VMEM((D, F), _BF16),
            pltpu.VMEM((NSLOT, B, W, Dh), _BF16),
            pltpu.VMEM((NSLOT, B, W, Dh), _BF16),
            pltpu.VMEM((Hkv, 2 * B, Dh), _F32),
            pltpu.VMEM((Hkv, 2 * B, Dh), _F32),
            pltpu.VMEM((B, D), A_x.dtype),
            pltpu.SemaphoreType.DMA((8,)),
            pltpu.SemaphoreType.DMA((2, NSLOT)),
            pltpu.SemaphoreType.DMA((2, GU_CH)),
            pltpu.SemaphoreType.DMA((n_wd,)),
        ],
        compiler_params=pltpu.CompilerParams(vmem_limit_bytes=100 * 1024 * 1024),
    )(A_x.reshape(B, D), A_k_cache, A_v_cache, A_wq, A_wo.T, B_w_r, B_w_gate,
      B_w_up, B_w_down.T, c, w_mod)
    return out.reshape(B, Sq, D)
```

```python
import jax
import jax.numpy as jnp
from jax import lax
import jax.experimental.pallas as pl
import jax.experimental.pallas.tpu as pltpu

_NT = (((1,), (1,)), ((), ()))
_NN = (((1,), (0,)), ((), ()))
_F32 = jnp.float32
_BF16 = jnp.bfloat16
HI, LO = 0, 1


def _layernorm(x, eps=1e-05):
    m = jnp.mean(x, axis=-1, keepdims=True)
    xc = x - m
    v = jnp.mean(xc * xc, axis=-1, keepdims=True)
    return xc / jnp.sqrt(v + eps)


def _sigmoid(x):
    return 1.0 / (1.0 + jnp.exp(-x))


def _dot(a, b, dims):
    return lax.dot_general(a, b, dims, preferred_element_type=_F32)


@jax.jit
def pallas_adaLN_cond__sliding_block_cached__moe_arch_mod__decode_kernel(
    A_x: jax.Array,
    A_k_cache: jax.Array,
    A_v_cache: jax.Array,
    A_wq: jax.Array,
    A_wo: jax.Array,
    B_x: jax.Array,
    B_w_r: jax.Array,
    B_w_gate: jax.Array,
    B_w_up: jax.Array,
    B_w_down: jax.Array,
    c: jax.Array,
    w_mod: jax.Array,
):
    B, Sq, D = A_x.shape
    _, Hkv, Sk, Dh = A_k_cache.shape
    Hq = A_wq.shape[1] // Dh
    F = B_w_gate.shape[1]
    W = min(4096, max(256, Sk // 4))
    rep = Hq // Hkv
    assert Sq == 1 and rep == 2 and B == 8 and Hkv == 16
    scale = float(Dh) ** -0.5

    HG = 8
    GPB = Hkv // HG
    NG = B * GPB
    PR = 16
    NP = W // PR
    NSL = D // 8
    LEAD = NSL
    NKS, NVS = 2, 3
    QROWS = rep * HG
    PRE = 8
    assert NP * PR == W and NSL * 8 == D

    def kernel(x_hbm, k_hbm, v_hbm, wq_hbm, wot_hbm, wr_hbm, wg_hbm, wu_hbm,
               wdt_hbm, c_hbm, wmod_hbm, out_hbm,
               xbuf, cbuf, wrbuf, wmodbuf, wqbuf, wotbuf, wgbuf, wubuf, wdtbuf,
               kvbuf, qs, os_, obuf,
               misc_sems, w_sems, kv_sems):
        cp_x = pltpu.make_async_copy(x_hbm, xbuf, misc_sems.at[0])
        cp_c = pltpu.make_async_copy(c_hbm, cbuf, misc_sems.at[1])
        cp_wr = pltpu.make_async_copy(wr_hbm, wrbuf, misc_sems.at[2])
        cp_out = pltpu.make_async_copy(obuf, out_hbm, misc_sems.at[3])

        weights = {
            'mod': (wmod_hbm, wmodbuf, 0, 1664),
            'q': (wq_hbm, wqbuf, 1, 2048),
            'o': (wot_hbm, wotbuf, 2, 2048),
            'g': (wg_hbm, wgbuf, 3, 2304),
            'u': (wu_hbm, wubuf, 4, 2304),
            'd': (wdt_hbm, wdtbuf, 5, 2304),
        }

        def w_start(name, prio, i):
            hbm, buf, s, split = weights[name]
            n = buf.shape[1]
            slab = (i % 4) * (NSL // 4) + i // 4
            rows = pl.ds(pl.multiple_of(slab * 8, 8), 8)
            cols = pl.ds(0, split) if prio == HI else pl.ds(split, n - split)
            pltpu.make_async_copy(hbm.at[rows, cols], buf.at[rows, cols],
                                  w_sems.at[s]).start(priority=prio)

        def w_wait(name):
            _, buf, s, _ = weights[name]
            pltpu.make_async_copy(buf, buf, w_sems.at[s]).wait()

        def kslot(g):
            return g % NKS

        def vslot(g):
            return NKS + g % NVS

        def kv_start(hbm, slot, g, u, prio):
            b = g // GPB
            h0 = (g % GPB) * HG
            r = pl.multiple_of(u * PR, PR)
            pltpu.make_async_copy(
                hbm.at[b, pl.ds(h0, HG), pl.ds(Sk - W + r, PR), :],
                kvbuf.at[slot, :, pl.ds(r, PR), :],
                kv_sems.at[slot]).start(priority=prio)

        def k_start(g, u):
            kv_start(k_hbm, kslot(g), g, u, HI)

        def v_start(i):
            g = i // NP
            kv_start(v_hbm, vslot(g), g, i % NP, LO)

        def kv_wait(slot):
            pltpu.make_async_copy(kvbuf.at[slot], kvbuf.at[slot], kv_sems.at[slot]).wait()

        def issue_loop(lo, hi, step_fn):
            def body(i, carry):
                step_fn(i)
                return carry
            lax.fori_loop(lo, hi, body, 0)

        def kv_step(g):
            def f(u):
                v_start(g * NP + u + LEAD)
                k_start(g, u)
            return f

        cp_c.start()
        cp_x.start()
        cp_wr.start()
        issue_loop(0, NSL, lambda i: w_start('mod', LO, i))

        def ww_step(lo_name, hi_name):
            def f(i):
                w_start(lo_name, LO, i)
                w_start(hi_name, HI, i)
            return f

        issue_loop(0, NSL, ww_step('q', 'mod'))
        issue_loop(0, NSL, ww_step('o', 'q'))

        def ov_step(i):
            v_start(i)
            w_start('o', HI, i)

        issue_loop(0, 8, ov_step)
        cp_c.wait()
        cp_x.wait()
        cf = cbuf[...].astype(_F32)
        sc = (cf * _sigmoid(cf)).astype(_BF16)
        xf = xbuf[...].astype(_F32)
        xn = _layernorm(xf)
        w_wait('mod')
        mod0 = _dot(sc, wmodbuf[:, pl.ds(0, 2 * D)], _NN)
        h1 = (xn * (1.0 + mod0[:, D:2 * D]) + mod0[:, 0:D]).astype(_BF16)
        issue_loop(8, 24, ov_step)
        w_wait('q')
        QC = 4
        for qc in range(QC):
            ncol = Hq * Dh // QC
            q = _dot(h1, wqbuf[:, pl.ds(qc * ncol, ncol)], _NN)
            for j in range(Hq // QC):
                hq = qc * (Hq // QC) + j
                qs[pl.ds(hq, B, stride=Hq), :] = q[:, j * Dh:(j + 1) * Dh]
            issue_loop(24 + 12 * qc, 36 + 12 * qc, ov_step)

        row2 = lax.broadcasted_iota(jnp.int32, (QROWS, Dh), 0) // rep

        def attend(g, step_fn):
            ks, vs = kslot(g), vslot(g)
            q16 = qs[pl.ds(pl.multiple_of(g * QROWS, QROWS), QROWS), :]
            kv_wait(ks)
            kv_wait(vs)
            half = W // 2
            s_h = [None, None]
            n = 0
            for j in range(HG):
                qj = jnp.where(row2 == j, q16, 0.0).astype(_BF16)
                for hh in range(2):
                    sj = _dot(qj, kvbuf[ks, j, pl.ds(hh * half, half), :], _NT)
                    s_h[hh] = sj if s_h[hh] is None else s_h[hh] + sj
                    step_fn(n)
                    n += 1
            s = jnp.concatenate(s_h, axis=1) * scale
            m = jnp.max(s, axis=-1, keepdims=True)
            p = jnp.exp(s - m)
            l = jnp.sum(p, axis=-1, keepdims=True)
            pb = p.astype(_BF16)
            o = jnp.zeros((QROWS, Dh), _F32)
            for j in range(HG):
                oj = _dot(pb, kvbuf[vs, j], _NN)
                o = jnp.where(row2 == j, oj, o)
                step_fn(n)
                n += 1
            os_[pl.ds(pl.multiple_of(g * QROWS, QROWS), QROWS), :] = o / l

        NINT = 3 * HG

        issue_loop(0, NP, kv_step(0))

        def period(t, carry):
            step = kv_step(t)
            issue_loop(0, PRE, step)
            attend(t - 1, lambda k: step(PRE + k))
            last = jnp.where(t == NG - 1, NP - LEAD, NP)
            issue_loop(PRE + NINT, last, step)
            return carry

        lax.fori_loop(1, NG, period, 0)

        def kg_step(i):
            w_start('g', LO, i)
            k_start(NG - 1, NP - LEAD + i)

        issue_loop(0, NSL, kg_step)

        gu = ww_step('u', 'g')
        issue_loop(0, PRE, gu)
        attend(NG - 1, lambda k: None)
        issue_loop(PRE, 40, gu)

        o_all = jnp.concatenate(
            [os_[pl.ds(hq, B, stride=Hq), :] for hq in range(Hq)], axis=1).astype(_BF16)
        w_wait('o')
        attn = _dot(o_all, wotbuf[...], _NT)
        issue_loop(40, 56, gu)
        mod1 = _dot(sc, wmodbuf[:, pl.ds(2 * D, 4 * D)], _NN)
        ga = mod1[:, 0:D]
        sb_ = mod1[:, D:2 * D]
        cb = mod1[:, 2 * D:3 * D]
        gb = mod1[:, 3 * D:4 * D]
        x1 = xf + ga * attn
        h2 = _layernorm(x1) * (1.0 + cb) + sb_
        h2b = h2.astype(_BF16)
        cp_wr.wait()
        wr = wrbuf[...].astype(_F32).reshape(1, D)
        r_sel = _sigmoid(jnp.sum(h2b.astype(_F32) * wr, axis=-1, keepdims=True))
        issue_loop(56, NSL, gu)

        ud = ww_step('d', 'u')
        issue_loop(0, PRE, ud)
        w_wait('g')
        g = _dot(h2b, wgbuf[...], _NN)
        sg = g * _sigmoid(g)
        issue_loop(PRE, NSL, ud)
        issue_loop(0, NSL, lambda i: w_start('d', HI, i))
        w_wait('u')
        u = _dot(h2b, wubuf[...], _NN)
        act = (sg * u).astype(_BF16)
        w_wait('d')
        y = _dot(act, wdtbuf[...], _NT)
        out = x1 + gb * (h2 + (h2 * 0.0 + y * r_sel))
        obuf[...] = out.astype(obuf.dtype)
        cp_out.start()
        cp_out.wait()

    any_spec = pl.BlockSpec(memory_space=pl.ANY)
    out = pl.pallas_call(
        kernel,
        out_shape=jax.ShapeDtypeStruct((B, D), A_x.dtype),
        in_specs=[any_spec] * 11,
        out_specs=any_spec,
        scratch_shapes=[
            pltpu.VMEM((B, D), _BF16),
            pltpu.VMEM((B, D), _BF16),
            pltpu.VMEM((D,), _BF16),
            pltpu.VMEM((D, 6 * D), _BF16),
            pltpu.VMEM((D, Hq * Dh), _BF16),
            pltpu.VMEM((D, Hq * Dh), _BF16),
            pltpu.VMEM((D, F), _BF16),
            pltpu.VMEM((D, F), _BF16),
            pltpu.VMEM((D, F), _BF16),
            pltpu.VMEM((NKS + NVS, HG, W, Dh), _BF16),
            pltpu.VMEM((B * Hq, Dh), _F32),
            pltpu.VMEM((B * Hq, Dh), _F32),
            pltpu.VMEM((B, D), A_x.dtype),
            pltpu.SemaphoreType.DMA((4,)),
            pltpu.SemaphoreType.DMA((6,)),
            pltpu.SemaphoreType.DMA((NKS + NVS,)),
        ],
        compiler_params=pltpu.CompilerParams(
            vmem_limit_bytes=100 * 1024 * 1024, disable_bounds_checks=True),
    )(A_x.reshape(B, D), A_k_cache, A_v_cache, A_wq, A_wo.T, B_w_r, B_w_gate,
      B_w_up, B_w_down.T, c, w_mod)
    return out.reshape(B, Sq, D)
```

```python
import jax
import jax.numpy as jnp
from jax import lax
import jax.experimental.pallas as pl
import jax.experimental.pallas.tpu as pltpu

_NT = (((1,), (1,)), ((), ()))
_NN = (((1,), (0,)), ((), ()))
_F32 = jnp.float32
_BF16 = jnp.bfloat16
HI, LO = 0, 1


def _layernorm(x, eps=1e-05):
    m = jnp.mean(x, axis=-1, keepdims=True)
    xc = x - m
    v = jnp.mean(xc * xc, axis=-1, keepdims=True)
    return xc / jnp.sqrt(v + eps)


def _sigmoid(x):
    return 1.0 / (1.0 + jnp.exp(-x))


def _dot(a, b, dims):
    return lax.dot_general(a, b, dims, preferred_element_type=_F32)


@jax.jit
def pallas_adaLN_cond__sliding_block_cached__moe_arch_mod__decode_kernel(
    A_x: jax.Array,
    A_k_cache: jax.Array,
    A_v_cache: jax.Array,
    A_wq: jax.Array,
    A_wo: jax.Array,
    B_x: jax.Array,
    B_w_r: jax.Array,
    B_w_gate: jax.Array,
    B_w_up: jax.Array,
    B_w_down: jax.Array,
    c: jax.Array,
    w_mod: jax.Array,
):
    B, Sq, D = A_x.shape
    _, Hkv, Sk, Dh = A_k_cache.shape
    Hq = A_wq.shape[1] // Dh
    F = B_w_gate.shape[1]
    W = min(4096, max(256, Sk // 4))
    rep = Hq // Hkv
    assert Sq == 1 and rep == 2 and B == 8 and Hkv == 16
    scale = float(Dh) ** -0.5

    HG = 8
    GPB = Hkv // HG
    NG = B * GPB
    PR = 16
    NP = W // PR
    NSL = D // 8
    LEAD = NSL
    NKS, NVS = 2, 3
    QROWS = rep * HG
    PRE = 8
    HOP = 4
    NOCOMP = False
    NOATT = False
    NOSEMCHK = True
    DLEAD = 16
    CHUNKED = True
    assert NP * PR == W and NSL * 8 == D
    DBLK = (0, 16, 32, 48, 64, 72)
    NDB = len(DBLK) - 1

    def kernel(x_hbm, k_hbm, v_hbm, wq_hbm, wot_hbm, wr_hbm, wg_hbm, wu_hbm,
               wdt_hbm, c_hbm, wmod_hbm, out_hbm,
               xbuf, cbuf, wrbuf, wmodbuf, wqbuf, wotbuf, wgbuf, wubuf, wdtbuf,
               kvbuf, qs, os_, obuf,
               misc_sems, w_sems, kv_sems, d_sems):
        cp_x = pltpu.make_async_copy(x_hbm, xbuf, misc_sems.at[0])
        cp_c = pltpu.make_async_copy(c_hbm, cbuf, misc_sems.at[1])
        cp_wr = pltpu.make_async_copy(wr_hbm, wrbuf, misc_sems.at[2])
        cp_out = pltpu.make_async_copy(obuf, out_hbm, misc_sems.at[3])

        weights = {
            'mod': (wmod_hbm, wmodbuf, 0, 1664),
            'q': (wq_hbm, wqbuf, 1, 2048),
            'o': (wot_hbm, wotbuf, 2, 2048),
            'g': (wg_hbm, wgbuf, 3, 2304),
            'u': (wu_hbm, wubuf, 4, 2304),
        }

        def w_start(name, prio, i):
            hbm, buf, s, split = weights[name]
            n = buf.shape[1]
            slab = (i % HOP) * (NSL // HOP) + i // HOP
            rows = pl.ds(pl.multiple_of(slab * 8, 8), 8)
            cols = pl.ds(0, split) if prio == HI else pl.ds(split, n - split)
            pltpu.make_async_copy(hbm.at[rows, cols], buf.at[rows, cols],
                                  w_sems.at[s]).start(priority=prio)

        def w_wait(name):
            _, buf, s, _ = weights[name]
            pltpu.make_async_copy(buf, buf, w_sems.at[s]).wait()

        def d_copy(prio, i):
            rows = pl.ds(pl.multiple_of(i * 8, 8), 8)
            cols = pl.ds(0 if prio == HI else F // 2, F // 2)
            return pltpu.make_async_copy(wdt_hbm.at[rows, cols], wdtbuf.at[rows, cols],
                                         d_sems.at[i // 16])

        def kslot(g):
            return g % NKS

        def vslot(g):
            return NKS + g % NVS

        def kv_start(hbm, slot, g, u, prio):
            b = g // GPB
            h0 = (g % GPB) * HG
            r = pl.multiple_of(u * PR, PR)
            pltpu.make_async_copy(
                hbm.at[b, pl.ds(h0, HG), pl.ds(Sk - W + r, PR), :],
                kvbuf.at[slot, :, pl.ds(r, PR), :],
                kv_sems.at[slot]).start(priority=prio)

        def k_start(g, u):
            kv_start(k_hbm, kslot(g), g, u, HI)

        def v_start(i):
            g = i // NP
            kv_start(v_hbm, vslot(g), g, i % NP, LO)

        def kv_wait(slot):
            pltpu.make_async_copy(kvbuf.at[slot], kvbuf.at[slot], kv_sems.at[slot]).wait()

        def issue_loop(lo, hi, step_fn):
            def body(i, carry):
                step_fn(i)
                return carry
            lax.fori_loop(lo, hi, body, 0)

        class Cursor:
            def __init__(self, segs):
                self.segs, self.s, self.i = segs, 0, 0

            def issue(self, n):
                while n > 0 and self.s < len(self.segs):
                    fn, cnt = self.segs[self.s]
                    m = min(n, cnt - self.i)
                    issue_loop(self.i, self.i + m, fn)
                    self.i += m
                    n -= m
                    if self.i == cnt:
                        self.s, self.i = self.s + 1, 0

            def finish_segment(self, s):
                while self.s <= s:
                    self.issue(self.segs[self.s][1] - self.i)

        def kv_step(g):
            def f(u):
                v_start(g * NP + u + LEAD)
                k_start(g, u)
            return f

        def ww_step(lo_name, hi_name):
            def f(i):
                w_start(lo_name, LO, i)
                w_start(hi_name, HI, i)
            return f

        def ov_step(i):
            v_start(i)
            w_start('o', HI, i)

        cp_c.start()
        cp_x.start()
        cp_wr.start()
        cur = Cursor([(lambda i: w_start('mod', LO, i), NSL),
                      (ww_step('q', 'mod'), NSL),
                      (ww_step('o', 'q'), NSL),
                      (ov_step, NSL),
                      (kv_step(0), NP)])
        cur.finish_segment(1)
        cur.issue(8)
        cp_c.wait()
        cp_x.wait()
        cf = cbuf[...].astype(_F32)
        sc = (cf * _sigmoid(cf)).astype(_BF16)
        xf = xbuf[...].astype(_F32)
        xn = _layernorm(xf)
        w_wait('mod')
        if not NOCOMP:
            MC = 9 if CHUNKED else 1
            mods = []
            for mc in range(MC):
                ncol = 6 * D // MC
                mods.append(_dot(sc, wmodbuf[:, pl.ds(mc * ncol, ncol)], _NN))
                cur.issue(4)
            mod = jnp.concatenate(mods, axis=1)
            h1 = (xn * (1.0 + mod[:, D:2 * D]) + mod[:, 0:D]).astype(_BF16)
            ga = mod[:, 2 * D:3 * D]
            sb_ = mod[:, 3 * D:4 * D]
            cb = mod[:, 4 * D:5 * D]
            gb = mod[:, 5 * D:6 * D]
        cur.finish_segment(2)
        cur.issue(8)
        w_wait('q')
        if not NOCOMP:
            QC = 8 if CHUNKED else 4
            for qc in range(QC):
                ncol = Hq * Dh // QC
                q = _dot(h1, wqbuf[:, pl.ds(qc * ncol, ncol)], _NN)
                for j in range(Hq // QC):
                    hq = qc * (Hq // QC) + j
                    qs[pl.ds(hq, B, stride=Hq), :] = q[:, j * Dh:(j + 1) * Dh]
                cur.issue(4)
        cur.finish_segment(4)

        row2 = lax.broadcasted_iota(jnp.int32, (QROWS, Dh), 0) // rep

        def attend(g, step_fn, skip=False):
            ks, vs = kslot(g), vslot(g)
            kv_wait(ks)
            kv_wait(vs)
            if skip:
                for n in range(3 * HG):
                    step_fn(n)
                return
            q16 = qs[pl.ds(pl.multiple_of(g * QROWS, QROWS), QROWS), :]
            half = W // 2
            s_h = [None, None]
            n = 0
            for j in range(HG):
                qj = jnp.where(row2 == j, q16, 0.0).astype(_BF16)
                for hh in range(2):
                    sj = _dot(qj, kvbuf[ks, j, pl.ds(hh * half, half), :], _NT)
                    s_h[hh] = sj if s_h[hh] is None else s_h[hh] + sj
                    step_fn(n)
                    n += 1
            s = jnp.concatenate(s_h, axis=1) * scale
            m = jnp.max(s, axis=-1, keepdims=True)
            p = jnp.exp(s - m)
            l = jnp.sum(p, axis=-1, keepdims=True)
            pb = p.astype(_BF16)
            o = jnp.zeros((QROWS, Dh), _F32)
            for j in range(HG):
                oj = _dot(pb, kvbuf[vs, j], _NN)
                o = jnp.where(row2 == j, oj, o)
                step_fn(n)
                n += 1
            os_[pl.ds(pl.multiple_of(g * QROWS, QROWS), QROWS), :] = o / l

        NINT = 3 * HG

        def period(t, carry):
            step = kv_step(t)
            issue_loop(0, PRE, step)
            attend(t - 1, lambda k: step(PRE + k), NOATT)
            last = jnp.where(t == NG - 1, NP - LEAD, NP)
            issue_loop(PRE + NINT, last, step)
            return carry

        lax.fori_loop(1, NG, period, 0)

        def kg_step(i):
            w_start('g', LO, i)
            k_start(NG - 1, NP - LEAD + i)

        def du_step(i):
            d_copy(LO, i).start(priority=LO)
            w_start('u', HI, i)

        def dd_step(i):
            d_copy(LO, i).wait()
            d_copy(HI, i).wait()
            d_copy(HI, i + DLEAD).start(priority=HI)

        def dw_step(i):
            d_copy(LO, i + NSL - DLEAD).wait()
            d_copy(HI, i + NSL - DLEAD).wait()

        cur = Cursor([(kg_step, NSL),
                      (ww_step('u', 'g'), NSL),
                      (du_step, NSL),
                      (lambda i: d_copy(HI, i).start(priority=HI), DLEAD),
                      (dd_step, NSL - DLEAD),
                      (dw_step, DLEAD)])
        cur.finish_segment(0)

        cur.issue(PRE)
        attend(NG - 1, (lambda k: cur.issue(2) if k % 2 == 1 or k >= 16 else None)
               if CHUNKED else (lambda k: None), NOCOMP)
        cur.issue(4)

        w_wait('o')
        cp_wr.wait()
        if not NOCOMP:
            o_all = jnp.concatenate(
                [os_[pl.ds(hq, B, stride=Hq), :] for hq in range(Hq)], axis=1).astype(_BF16)
            OC = 8 if CHUNKED else 1
            attn = None
            for oc in range(OC):
                ncol = Hq * Dh // OC
                a = _dot(o_all[:, oc * ncol:(oc + 1) * ncol],
                         wotbuf[:, pl.ds(oc * ncol, ncol)], _NT)
                attn = a if attn is None else attn + a
                cur.issue(3)
            x1 = xf + ga * attn
            h2 = _layernorm(x1) * (1.0 + cb) + sb_
            h2b = h2.astype(_BF16)
            wr = wrbuf[...].astype(_F32).reshape(1, D)
            r_sel = _sigmoid(jnp.sum(h2b.astype(_F32) * wr, axis=-1, keepdims=True))
        cur.finish_segment(1)

        cur.issue(PRE)
        w_wait('g')
        FC = 9 if CHUNKED else 1
        fcol = F // FC
        if not NOCOMP:
            sgs = []
            for fc in range(FC):
                g = _dot(h2b, wgbuf[:, pl.ds(fc * fcol, fcol)], _NN)
                sgs.append(g * _sigmoid(g))
                cur.issue(3)
        cur.finish_segment(3)
        cur.issue(3)
        w_wait('u')
        if not NOCOMP:
            acts = []
            for fc in range(FC):
                u = _dot(h2b, wubuf[:, pl.ds(fc * fcol, fcol)], _NN)
                acts.append((sgs[fc] * u).astype(_BF16))
                cur.issue(2)
            act = jnp.concatenate(acts, axis=1)
        ys = []
        for db in range(NDB):
            done = cur.i if cur.s == 4 else (NSL - DLEAD + cur.i if cur.s == 5 else NSL)
            if done < DBLK[db + 1]:
                cur.issue(DBLK[db + 1] - done)
            if not NOCOMP:
                r0, r1 = DBLK[db] * 8, DBLK[db + 1] * 8
                ys.append(_dot(act, wdtbuf[pl.ds(r0, r1 - r0), :], _NT))
        if not NOCOMP:
            y = jnp.concatenate(ys, axis=1)
            out = x1 + gb * (h2 + (h2 * 0.0 + y * r_sel))
        else:
            out = xf
        obuf[...] = out.astype(obuf.dtype)
        cp_out.start()
        cp_out.wait()

    any_spec = pl.BlockSpec(memory_space=pl.ANY)
    out = pl.pallas_call(
        kernel,
        out_shape=jax.ShapeDtypeStruct((B, D), A_x.dtype),
        in_specs=[any_spec] * 11,
        out_specs=any_spec,
        scratch_shapes=[
            pltpu.VMEM((B, D), _BF16),
            pltpu.VMEM((B, D), _BF16),
            pltpu.VMEM((D,), _BF16),
            pltpu.VMEM((D, 6 * D), _BF16),
            pltpu.VMEM((D, Hq * Dh), _BF16),
            pltpu.VMEM((D, Hq * Dh), _BF16),
            pltpu.VMEM((D, F), _BF16),
            pltpu.VMEM((D, F), _BF16),
            pltpu.VMEM((D, F), _BF16),
            pltpu.VMEM((NKS + NVS, HG, W, Dh), _BF16),
            pltpu.VMEM((B * Hq, Dh), _F32),
            pltpu.VMEM((B * Hq, Dh), _F32),
            pltpu.VMEM((B, D), A_x.dtype),
            pltpu.SemaphoreType.DMA((4,)),
            pltpu.SemaphoreType.DMA((5,)),
            pltpu.SemaphoreType.DMA((NKS + NVS,)),
            pltpu.SemaphoreType.DMA((NDB,)),
        ],
        compiler_params=pltpu.CompilerParams(
            vmem_limit_bytes=100 * 1024 * 1024, disable_bounds_checks=True,
            disable_semaphore_checks=NOSEMCHK),
    )(A_x.reshape(B, D), A_k_cache, A_v_cache, A_wq, A_wo.T, B_w_r, B_w_gate,
      B_w_up, B_w_down.T, c, w_mod)
    return out.reshape(B, Sq, D)
```

```python
import jax
import jax.numpy as jnp
from jax import lax
import jax.experimental.pallas as pl
import jax.experimental.pallas.tpu as pltpu

_NT = (((1,), (1,)), ((), ()))
_NN = (((1,), (0,)), ((), ()))
_F32 = jnp.float32
_BF16 = jnp.bfloat16
HI, LO = 0, 1


def _layernorm(x, eps=1e-05):
    m = jnp.mean(x, axis=-1, keepdims=True)
    xc = x - m
    v = jnp.mean(xc * xc, axis=-1, keepdims=True)
    return xc / jnp.sqrt(v + eps)


def _sigmoid(x):
    return 1.0 / (1.0 + jnp.exp(-x))


def _dot(a, b, dims):
    return lax.dot_general(a, b, dims, preferred_element_type=_F32)


class _NoScope:
    def __enter__(self):
        return self

    def __exit__(self, *a):
        return False


@jax.jit
def pallas_adaLN_cond__sliding_block_cached__moe_arch_mod__decode_kernel(
    A_x: jax.Array,
    A_k_cache: jax.Array,
    A_v_cache: jax.Array,
    A_wq: jax.Array,
    A_wo: jax.Array,
    B_x: jax.Array,
    B_w_r: jax.Array,
    B_w_gate: jax.Array,
    B_w_up: jax.Array,
    B_w_down: jax.Array,
    c: jax.Array,
    w_mod: jax.Array,
):
    B, Sq, D = A_x.shape
    _, Hkv, Sk, Dh = A_k_cache.shape
    Hq = A_wq.shape[1] // Dh
    F = B_w_gate.shape[1]
    W = min(4096, max(256, Sk // 4))
    rep = Hq // Hkv
    assert Sq == 1 and rep == 2 and B == 8 and Hkv == 16
    scale = float(Dh) ** -0.5

    HG = 8
    GPB = Hkv // HG
    NG = B * GPB
    PR = 16
    NP = W // PR
    NSL = D // 8
    NKS, NVS = 2, 2
    QROWS = rep * HG
    FH = F // 2
    LEAD = 0
    LAG = 60
    HOP = 4
    RHOP = 4
    NOCOMP = False
    SCOPES = False
    LCH = (8, 6, 4)
    HIGRP = ((0, 2), (2, 2), (4, 1))
    LOGRP = ((0, 2), (2, 1), (4, 1))
    INTER = True
    REFILL = 16
    assert NP * PR == W and NSL * 8 == D
    DBLK = (0, 16, 32, 48, 64, 72)
    NDB = len(DBLK) - 1
    LB = 3
    assert sum(LCH) * 128 == FH
    NINT = 3 * HG if INTER else 0
    assert LAG + NINT <= NP - LEAD

    def scope(name):
        return jax.named_scope(name) if SCOPES else _NoScope()

    def kernel(x_hbm, k_hbm, v_hbm, wq_hbm, wot_hbm, wr_hbm, wg_hbm, wu_hbm,
               wdt_hbm, c_hbm, wmod_hbm, out_hbm,
               xbuf, cbuf, wrbuf, wmodbuf, wqbuf, wotbuf, wgbuf, wubuf, wdtbuf,
               kvbuf, qs, os_, ep, obuf,
               misc_sems, w_sems, kv_sems, d_sems):
        cp_x = pltpu.make_async_copy(x_hbm, xbuf, misc_sems.at[0])
        cp_c = pltpu.make_async_copy(c_hbm, cbuf, misc_sems.at[1])
        cp_wr = pltpu.make_async_copy(wr_hbm, wrbuf, misc_sems.at[2])
        cp_out = pltpu.make_async_copy(obuf, out_hbm, misc_sems.at[3])

        weights = {
            'mod': (wmod_hbm, wmodbuf, 0, 1664),
            'q': (wq_hbm, wqbuf, 1, 2048),
            'o': (wot_hbm, wotbuf, 2, 2048),
            'g': (wg_hbm, wgbuf, 3, 2304),
            'u': (wu_hbm, wubuf, 4, 2304),
        }

        def w_start(name, prio):
            hbm, buf, s, split = weights[name]
            n = buf.shape[1]

            def f(i):
                if 2 * split == n:
                    p = i // RHOP
                    slab = ((0 if prio == HI else NSL // 2)
                            + (i % RHOP) * (NSL // 2 // RHOP) + p // 2)
                    cols = pl.ds(pl.multiple_of((p % 2) * split, 128), split)
                else:
                    slab = (i % HOP) * (NSL // HOP) + i // HOP
                    cols = pl.ds(0, split) if prio == HI else pl.ds(split, n - split)
                rows = pl.ds(pl.multiple_of(slab * 8, 8), 8)
                pltpu.make_async_copy(hbm.at[rows, cols], buf.at[rows, cols],
                                      w_sems.at[s]).start(priority=prio)
            return f

        def w_wait(name):
            _, buf, s, _ = weights[name]
            with scope('wait_' + name):
                pltpu.make_async_copy(buf, buf, w_sems.at[s]).wait()

        def d_rows(prio, b0, nb):
            def f(i):
                blk = b0 + i % nb if nb > 1 else b0
                rows = pl.ds(pl.multiple_of((blk * 16 + i // nb) * 8, 8), 8)
                cols = pl.ds(0 if prio == HI else FH, FH)
                pltpu.make_async_copy(wdt_hbm.at[rows, cols], wdtbuf.at[rows, cols],
                                      d_sems.at[prio, blk]).start(priority=prio)
            return f, sum(DBLK[b + 1] - DBLK[b] for b in range(b0, b0 + nb))

        def d_cols(k):
            c0 = sum(LCH[:k])

            def f(i):
                sl = (pl.ds(LB * 128, 128),
                      pl.ds(pl.multiple_of(FH + (c0 + i) * 128, 128), 128))
                pltpu.make_async_copy(wdt_hbm.at[sl], wdtbuf.at[sl],
                                      d_sems.at[2, k]).start(priority=LO)
            return f, LCH[k]

        def d_unit(name):
            kind, n = name[0], int(name[1])
            if kind == 'C':
                c0 = FH + sum(LCH[:n]) * 128
                return (LB * 128, LB * 128 + 128), (c0, c0 + LCH[n] * 128), d_sems.at[2, n]
            prio = HI if kind == 'L' else LO
            return ((DBLK[n] * 8, DBLK[n + 1] * 8), (0, FH) if kind == 'L' else (FH, F),
                    d_sems.at[prio, n])

        def kslot(g):
            return g % NKS

        def vslot(g):
            return NKS + g % NVS

        def kv_start(hbm, slot_fn, prio):
            def f(i):
                g = i // NP
                r = pl.multiple_of((i % NP) * PR, PR)
                slot = slot_fn(g)
                pltpu.make_async_copy(
                    hbm.at[pl.ds(g * HG, HG), pl.ds(Sk - W + r, PR), :],
                    kvbuf.at[slot, :, pl.ds(r, PR), :],
                    kv_sems.at[slot]).start(priority=prio)
            return f

        k_start = kv_start(k_hbm, kslot, HI)
        v_start = kv_start(v_hbm, vslot, LO)

        def kv_wait(slot):
            pltpu.make_async_copy(kvbuf.at[slot], kvbuf.at[slot], kv_sems.at[slot]).wait()

        def issue_loop(lo, hi, step_fn):
            def body(i, carry):
                step_fn(i)
                return carry
            lax.fori_loop(lo, hi, body, 0)

        hi_segs = [(None, LEAD), (w_start('mod', HI), NSL), (w_start('q', HI), NSL),
                   (w_start('o', HI), NSL), (k_start, NG * NP), (w_start('g', HI), NSL),
                   (w_start('u', HI), NSL)] + [d_rows(HI, *a) for a in HIGRP]
        lo_segs = [(w_start('mod', LO), NSL), (w_start('q', LO), NSL),
                   (w_start('o', LO), NSL), (v_start, NG * NP), (w_start('g', LO), NSL),
                   (w_start('u', LO), NSL)] + [d_rows(LO, *a) for a in LOGRP]
        lo_segs += [d_cols(k) for k in range(len(LCH))]
        KV0 = LEAD + 3 * NSL
        KV1 = KV0 + NG * NP
        TOTAL = max(sum(n for _, n in hi_segs), sum(n for _, n in lo_segs))

        def locate(segs, pos):
            for fn, n in segs:
                if pos < n:
                    return fn, pos, n - pos
                pos -= n
            return None, 0, TOTAL

        state = {'pos': 0}

        def issue_to(target):
            target = min(target, TOTAL)
            while state['pos'] < target:
                pos = state['pos']
                lf, li, ln = locate(lo_segs, pos)
                hf, hi_, hn = locate(hi_segs, pos)
                m = min(target - pos, ln, hn)

                def step(i, lf=lf, li=li, hf=hf, hi_=hi_):
                    if lf is not None:
                        lf(li + i)
                    if hf is not None:
                        hf(hi_ + i)
                issue_loop(0, m, step)
                state['pos'] = pos + m

        def issue(n):
            issue_to(state['pos'] + n)

        cp_c.start()
        cp_x.start()
        cp_wr.start()
        issue_to(LEAD + NSL + LAG)
        cp_c.wait()
        cp_x.wait()
        cf = cbuf[...].astype(_F32)
        sc = (cf * _sigmoid(cf)).astype(_BF16)
        xf = xbuf[...].astype(_F32)
        xn = _layernorm(xf)
        w_wait('mod')
        if not NOCOMP:
            mod = _dot(sc, wmodbuf[...], _NN)
            h1 = (xn * (1.0 + mod[:, D:2 * D]) + mod[:, 0:D]).astype(_BF16)
            ga = mod[:, 2 * D:3 * D]
            sb_ = mod[:, 3 * D:4 * D]
            cb = mod[:, 4 * D:5 * D]
            gb = mod[:, 5 * D:6 * D]
        issue_to(LEAD + 2 * NSL + LAG)
        w_wait('q')
        if not NOCOMP:
            q = _dot(h1, wqbuf[...], _NN)
            for hq in range(Hq):
                qs[pl.ds(hq, B, stride=Hq), :] = q[:, hq * Dh:(hq + 1) * Dh]
        issue_to(KV0 + NP)

        row2 = lax.broadcasted_iota(jnp.int32, (QROWS, Dh), 0) // rep

        def attend(g, step_fn, mid_fn):
            ks, vs = kslot(g), vslot(g)
            with scope('wk'):
                kv_wait(ks)
            with scope('wv'):
                kv_wait(vs)
            if NOCOMP:
                for n in range(3 * HG):
                    step_fn(n)
                mid_fn()
                return
            q16 = qs[pl.ds(pl.multiple_of(g * QROWS, QROWS), QROWS), :]
            half = W // 2
            s_h = [None, None]
            n = 0
            for j in range(HG):
                qj = jnp.where(row2 == j, q16, 0.0).astype(_BF16)
                for hh in range(2):
                    sj = _dot(qj, kvbuf[ks, j, pl.ds(hh * half, half), :], _NT)
                    s_h[hh] = sj if s_h[hh] is None else sj + s_h[hh]
                    step_fn(n)
                    n += 1
            s = jnp.concatenate(s_h, axis=1) * scale
            m = jnp.max(s, axis=-1, keepdims=True)
            p = jnp.exp(s - m)
            l = jnp.sum(p, axis=-1, keepdims=True)
            pb = p.astype(_BF16)
            mid_fn()
            o = jnp.zeros((QROWS, Dh), _F32)
            for j in range(HG):
                oj = _dot(pb, kvbuf[vs, j], _NN)
                o = jnp.where(row2 == j, oj, o)
                step_fn(n)
                n += 1
            os_[pl.ds(pl.multiple_of(g * QROWS, QROWS), QROWS), :] = o / l

        def period(t, carry):
            def step(u):
                v_start(t * NP + u + LEAD)
                k_start(t * NP + u)
            issue_loop(0, LAG, step)
            if INTER:
                attend(t - 1, lambda k: step(LAG + k), lambda: None)
                done = LAG + NINT
            else:
                attend(t - 1, lambda k: None, lambda: issue_loop(LAG, LAG + 20, step))
                done = LAG + 20
            last = jnp.where(t == NG - 1, NP - LEAD, NP) if LEAD else NP
            with scope('rest'):
                issue_loop(done, last, step)
            return carry

        lax.fori_loop(1, NG, period, 0)
        state['pos'] = KV1 - LEAD

        issue_to(KV1 + LAG)
        with scope('att15'):
            attend(NG - 1, lambda k: None, lambda: issue(REFILL + 4))
        issue(REFILL)

        w_wait('o')
        cp_wr.wait()
        if not NOCOMP:
            o_all = jnp.concatenate(
                [os_[pl.ds(hq, B, stride=Hq), :] for hq in range(Hq)], axis=1).astype(_BF16)
            attn = _dot(o_all, wotbuf[...], _NT)
            x1 = xf + ga * attn
            h2 = _layernorm(x1) * (1.0 + cb) + sb_
            h2b = h2.astype(_BF16)
            wr = wrbuf[...].astype(_F32).reshape(1, D)
            r_sel = _sigmoid(jnp.sum(h2b.astype(_F32) * wr, axis=-1, keepdims=True))
            ep[0] = x1 + gb * (h2 + h2 * 0.0)
            ep[1] = gb * r_sel

        issue_to(max(KV1 + NSL + LAG, state['pos'] + REFILL))
        w_wait('g')
        if not NOCOMP:
            g = _dot(h2b, wgbuf[...], _NN)
            sg = g * _sigmoid(g)
        issue_to(KV1 + 2 * NSL + LAG)
        w_wait('u')
        if not NOCOMP:
            u = _dot(h2b, wubuf[...], _NN)
            act = (sg * u).astype(_BF16)
        with scope('lastissue'):
            issue_to(TOTAL)

        ORDER = 'L0 L1 R0 R1 L2 L3 L4 R2 R4 C0 C1 C2'
        units = ORDER.split()
        for n, name in enumerate(units):
            (r0, r1), (c0, c1), sem = d_unit(name)
            view = wdtbuf.at[pl.ds(r0, r1 - r0), pl.ds(c0, c1 - c0)]
            with scope('wait_' + name):
                pltpu.make_async_copy(view, view, sem).wait()
            cols = pl.ds(r0, r1 - r0)
            final = not any(d_unit(m)[0] == (r0, r1) for m in units[n + 1:])
            if NOCOMP:
                if final:
                    obuf[:, cols] = xbuf[:, cols]
                continue
            y = _dot(act[:, c0:c1], wdtbuf[cols, pl.ds(c0, c1 - c0)], _NT)
            acc = ep[0, :, cols] + ep[1, :, cols] * y
            if final:
                obuf[:, cols] = acc.astype(obuf.dtype)
            else:
                ep[0, :, cols] = acc
        with scope('out'):
            cp_out.start()
            cp_out.wait()

    any_spec = pl.BlockSpec(memory_space=pl.ANY)
    out = pl.pallas_call(
        kernel,
        out_shape=jax.ShapeDtypeStruct((B, D), A_x.dtype),
        in_specs=[any_spec] * 11,
        out_specs=any_spec,
        scratch_shapes=[
            pltpu.VMEM((B, D), _BF16),
            pltpu.VMEM((B, D), _BF16),
            pltpu.VMEM((D,), _BF16),
            pltpu.VMEM((D, 6 * D), _BF16),
            pltpu.VMEM((D, Hq * Dh), _BF16),
            pltpu.VMEM((D, Hq * Dh), _BF16),
            pltpu.VMEM((D, F), _BF16),
            pltpu.VMEM((D, F), _BF16),
            pltpu.VMEM((D, F), _BF16),
            pltpu.VMEM((NKS + NVS, HG, W, Dh), _BF16),
            pltpu.VMEM(((B + 1) * Hq, Dh), _F32),
            pltpu.VMEM(((B + 1) * Hq, Dh), _F32),
            pltpu.VMEM((2, B, D), _F32),
            pltpu.VMEM((B, D), A_x.dtype),
            pltpu.SemaphoreType.DMA((4,)),
            pltpu.SemaphoreType.DMA((5,)),
            pltpu.SemaphoreType.DMA((NKS + NVS,)),
            pltpu.SemaphoreType.DMA((3, NDB)),
        ],
        compiler_params=pltpu.CompilerParams(
            vmem_limit_bytes=100 * 1024 * 1024, disable_bounds_checks=True,
            disable_semaphore_checks=True),
    )(A_x.reshape(B, D), A_k_cache.reshape(B * Hkv, Sk, Dh),
      A_v_cache.reshape(B * Hkv, Sk, Dh), A_wq, A_wo.T, B_w_r, B_w_gate,
      B_w_up, B_w_down.T, c, w_mod)
    return out.reshape(B, Sq, D)
```

```python
import jax
import jax.numpy as jnp
from jax import lax
import jax.experimental.pallas as pl
import jax.experimental.pallas.tpu as pltpu

_NT = (((1,), (1,)), ((), ()))
_NN = (((1,), (0,)), ((), ()))
_F32 = jnp.float32
_BF16 = jnp.bfloat16
HI, LO = 0, 1


def _layernorm(x, eps=1e-05):
    m = jnp.mean(x, axis=-1, keepdims=True)
    xc = x - m
    v = jnp.mean(xc * xc, axis=-1, keepdims=True)
    return xc / jnp.sqrt(v + eps)


def _sigmoid(x):
    return 1.0 / (1.0 + jnp.exp(-x))


def _dot(a, b, dims):
    return lax.dot_general(a, b, dims, preferred_element_type=_F32)


@jax.jit
def pallas_adaLN_cond__sliding_block_cached__moe_arch_mod__decode_kernel(
    A_x: jax.Array,
    A_k_cache: jax.Array,
    A_v_cache: jax.Array,
    A_wq: jax.Array,
    A_wo: jax.Array,
    B_x: jax.Array,
    B_w_r: jax.Array,
    B_w_gate: jax.Array,
    B_w_up: jax.Array,
    B_w_down: jax.Array,
    c: jax.Array,
    w_mod: jax.Array,
):
    B, Sq, D = A_x.shape
    _, Hkv, Sk, Dh = A_k_cache.shape
    Hq = A_wq.shape[1] // Dh
    F = B_w_gate.shape[1]
    W = min(4096, max(256, Sk // 4))
    rep = Hq // Hkv
    assert (B, Sq, D, Hq, Hkv, Dh, F, W) == (8, 1, 576, 32, 16, 128, 4608, 2048)
    scale = float(Dh) ** -0.5

    HG = 8
    NG = B * Hkv // HG
    QROWS = rep * HG
    PR = 16
    NP = W // PR
    NSL = D // 8
    HOP = 4
    LAG = 60
    NINT = 3 * HG
    FH = F // 2
    DBLK = (0, 16, 32, 48, 64, 72)
    LB = 3
    LCH = (8, 6, 4)
    D_HI = ((0, 2), (2, 2), (4, 1))
    D_LO = ((0, 2), (2, 1), (4, 1))
    D_ORDER = 'L0 L1 R0 R1 L2 L3 L4 R2 R4 C0 C1 C2'.split()
    assert sum(LCH) * 128 == FH and LAG + NINT <= NP and LAG <= NSL

    def kernel(x_hbm, k_hbm, v_hbm, wq_hbm, wot_hbm, wr_hbm, wg_hbm, wu_hbm,
               wdt_hbm, c_hbm, wmod_hbm, out_hbm,
               xbuf, cbuf, wrbuf, wmodbuf, wqbuf, wotbuf, wgbuf, wubuf, wdtbuf,
               kvbuf, qs, os_, ep, obuf,
               misc_sems, w_sems, kv_sems, d_sems):
        cp_x = pltpu.make_async_copy(x_hbm, xbuf, misc_sems.at[0])
        cp_c = pltpu.make_async_copy(c_hbm, cbuf, misc_sems.at[1])
        cp_wr = pltpu.make_async_copy(wr_hbm, wrbuf, misc_sems.at[2])
        cp_out = pltpu.make_async_copy(obuf, out_hbm, misc_sems.at[3])

        weights = {
            'mod': (wmod_hbm, wmodbuf, 0, 13 * 128),
            'q': (wq_hbm, wqbuf, 1, Hq * Dh // 2),
            'o': (wot_hbm, wotbuf, 2, Hq * Dh // 2),
            'g': (wg_hbm, wgbuf, 3, FH),
            'u': (wu_hbm, wubuf, 4, FH),
        }

        def w_seg(name, prio):
            hbm, buf, s, split = weights[name]
            n = buf.shape[1]

            def start(i):
                if 2 * split == n:
                    p = i // HOP
                    slab = ((0 if prio == HI else NSL // 2)
                            + (i % HOP) * (NSL // 2 // HOP) + p // 2)
                    cols = pl.ds(pl.multiple_of((p % 2) * split, 128), split)
                else:
                    slab = (i % HOP) * (NSL // HOP) + i // HOP
                    cols = pl.ds(0, split) if prio == HI else pl.ds(split, n - split)
                rows = pl.ds(pl.multiple_of(slab * 8, 8), 8)
                pltpu.make_async_copy(hbm.at[rows, cols], buf.at[rows, cols],
                                      w_sems.at[s]).start(priority=prio)
            return start, NSL

        def w_wait(name):
            _, buf, s, _ = weights[name]
            pltpu.make_async_copy(buf, buf, w_sems.at[s]).wait()

        def d_rows_seg(prio, b0, nb):
            def start(i):
                blk = b0 + i % nb if nb > 1 else b0
                rows = pl.ds(pl.multiple_of((blk * 16 + i // nb) * 8, 8), 8)
                cols = pl.ds(0 if prio == HI else FH, FH)
                pltpu.make_async_copy(wdt_hbm.at[rows, cols], wdtbuf.at[rows, cols],
                                      d_sems.at[prio, blk]).start(priority=prio)
            return start, DBLK[b0 + nb] - DBLK[b0]

        def d_cols_seg(k):
            c0 = FH + sum(LCH[:k]) * 128

            def start(i):
                rows = pl.ds(pl.multiple_of(LB * 128 + (i % 2) * 64, 64), 64)
                cols = pl.ds(pl.multiple_of(c0 + (i // 2) * 256, 128), 256)
                pltpu.make_async_copy(wdt_hbm.at[rows, cols], wdtbuf.at[rows, cols],
                                      d_sems.at[2, k]).start(priority=LO)
            return start, LCH[k]

        def d_unit(name):
            kind, n = name[0], int(name[1])
            if kind == 'C':
                c0 = FH + sum(LCH[:n]) * 128
                return (LB * 128, LB * 128 + 128), (c0, c0 + LCH[n] * 128), d_sems.at[2, n]
            rows = (DBLK[n] * 8, DBLK[n + 1] * 8)
            if kind == 'L':
                return rows, (0, FH), d_sems.at[HI, n]
            return rows, (FH, F), d_sems.at[LO, n]

        def kslot(g):
            return g % 2

        def vslot(g):
            return 2 + g % 2

        def kv_step(g):
            def start(hbm, slot, u, prio):
                r = pl.multiple_of(u * PR, PR)
                pltpu.make_async_copy(
                    hbm.at[pl.ds(g * HG, HG), pl.ds(Sk - W + r, PR), :],
                    kvbuf.at[slot, :, pl.ds(r, PR), :],
                    kv_sems.at[slot]).start(priority=prio)

            def step(u):
                start(v_hbm, vslot(g), u, LO)
                start(k_hbm, kslot(g), u, HI)
            return step

        def kv_wait(slot):
            pltpu.make_async_copy(kvbuf.at[slot], kvbuf.at[slot], kv_sems.at[slot]).wait()

        def issue_loop(lo, hi, step):
            def body(i, carry):
                step(i)
                return carry
            lax.fori_loop(lo, hi, body, 0)

        def make_issuer(lo_segs, hi_segs):
            total = max(sum(n for _, n in lo_segs), sum(n for _, n in hi_segs))
            done = [0]

            def locate(segs, pos):
                for fn, n in segs:
                    if pos < n:
                        return fn, pos, n - pos
                    pos -= n
                return None, 0, total

            def issue_to(target):
                while done[0] < min(target, total):
                    lf, li, ln = locate(lo_segs, done[0])
                    hf, hi, hn = locate(hi_segs, done[0])
                    m = min(min(target, total) - done[0], ln, hn)

                    def step(i):
                        if lf is not None:
                            lf(li + i)
                        if hf is not None:
                            hf(hi + i)
                    issue_loop(0, m, step)
                    done[0] += m
            return issue_to, total

        cp_c.start()
        cp_x.start()
        cp_wr.start()
        issue_to, n_pre = make_issuer([w_seg(n, LO) for n in ('mod', 'q', 'o')],
                                      [w_seg(n, HI) for n in ('mod', 'q', 'o')])
        issue_to(NSL + LAG)
        cp_c.wait()
        cp_x.wait()
        cf = cbuf[...].astype(_F32)
        sc = (cf * _sigmoid(cf)).astype(_BF16)
        xf = xbuf[...].astype(_F32)
        xn = _layernorm(xf)
        w_wait('mod')
        mod = _dot(sc, wmodbuf[...], _NN)
        sa, ca, ga, sb, cb, gb = [mod[:, i * D:(i + 1) * D] for i in range(6)]
        h1 = (xn * (1.0 + ca) + sa).astype(_BF16)
        issue_to(2 * NSL + LAG)
        w_wait('q')
        q = _dot(h1, wqbuf[...], _NN)
        for hq in range(Hq):
            qs[pl.ds(hq, B, stride=Hq), :] = q[:, hq * Dh:(hq + 1) * Dh]
        issue_to(n_pre)
        issue_loop(0, NP, kv_step(0))

        qrow = lax.broadcasted_iota(jnp.int32, (QROWS, Dh), 0) // rep

        def attend(g, step, mid):
            ks, vs = kslot(g), vslot(g)
            rows = pl.ds(pl.multiple_of(g * QROWS, QROWS), QROWS)
            kv_wait(ks)
            kv_wait(vs)
            q16 = qs[rows, :]
            half = W // 2
            s_h = [None, None]
            for j in range(HG):
                qj = jnp.where(qrow == j, q16, 0.0).astype(_BF16)
                for hh in range(2):
                    sj = _dot(qj, kvbuf[ks, j, pl.ds(hh * half, half), :], _NT)
                    s_h[hh] = sj if s_h[hh] is None else sj + s_h[hh]
                    step(2 * j + hh)
            s = jnp.concatenate(s_h, axis=1) * scale
            m = jnp.max(s, axis=-1, keepdims=True)
            p = jnp.exp(s - m)
            l = jnp.sum(p, axis=-1, keepdims=True)
            pb = p.astype(_BF16)
            mid()
            o = jnp.zeros((QROWS, Dh), _F32)
            for j in range(HG):
                o = jnp.where(qrow == j, _dot(pb, kvbuf[vs, j], _NN), o)
                step(2 * HG + j)
            os_[rows, :] = o / l

        def period(t, carry):
            step = kv_step(t)
            issue_loop(0, LAG, step)
            attend(t - 1, lambda k: step(LAG + k), lambda: None)
            issue_loop(LAG + NINT, NP, step)
            return carry

        lax.fori_loop(1, NG, period, 0)

        issue_to, n_post = make_issuer(
            [w_seg('g', LO), w_seg('u', LO)] + [d_rows_seg(LO, *a) for a in D_LO]
            + [d_cols_seg(k) for k in range(len(LCH))],
            [w_seg('g', HI), w_seg('u', HI)] + [d_rows_seg(HI, *a) for a in D_HI])
        issue_to(LAG)
        attend(NG - 1, lambda k: None, lambda: issue_to(LAG + 20))
        issue_to(LAG + 36)

        w_wait('o')
        cp_wr.wait()
        o_all = jnp.concatenate(
            [os_[pl.ds(hq, B, stride=Hq), :] for hq in range(Hq)], axis=1).astype(_BF16)
        x1 = xf + ga * _dot(o_all, wotbuf[...], _NT)
        h2 = _layernorm(x1) * (1.0 + cb) + sb
        h2b = h2.astype(_BF16)
        wr = wrbuf[...].astype(_F32).reshape(1, D)
        r_sel = _sigmoid(jnp.sum(h2b.astype(_F32) * wr, axis=-1, keepdims=True))
        ep[0] = x1 + gb * (h2 + h2 * 0.0)
        ep[1] = gb * r_sel

        issue_to(NSL + LAG)
        w_wait('g')
        g = _dot(h2b, wgbuf[...], _NN)
        sg = g * _sigmoid(g)
        issue_to(2 * NSL + LAG)
        w_wait('u')
        act = (sg * _dot(h2b, wubuf[...], _NN)).astype(_BF16)
        issue_to(n_post)
        for n, name in enumerate(D_ORDER):
            (r0, r1), (c0, c1), sem = d_unit(name)
            rows, cols = pl.ds(r0, r1 - r0), pl.ds(c0, c1 - c0)
            pltpu.make_async_copy(wdtbuf.at[rows, cols], wdtbuf.at[rows, cols], sem).wait()
            y = _dot(act[:, c0:c1], wdtbuf[rows, cols], _NT)
            acc = ep[0, :, rows] + ep[1, :, rows] * y
            if any(d_unit(later)[0] == (r0, r1) for later in D_ORDER[n + 1:]):
                ep[0, :, rows] = acc
            else:
                obuf[:, rows] = acc.astype(obuf.dtype)
        cp_out.start()
        cp_out.wait()

    any_spec = pl.BlockSpec(memory_space=pl.ANY)
    out = pl.pallas_call(
        kernel,
        out_shape=jax.ShapeDtypeStruct((B, D), A_x.dtype),
        in_specs=[any_spec] * 11,
        out_specs=any_spec,
        scratch_shapes=[
            pltpu.VMEM((B, D), _BF16),
            pltpu.VMEM((B, D), _BF16),
            pltpu.VMEM((D,), _BF16),
            pltpu.VMEM((D, 6 * D), _BF16),
            pltpu.VMEM((D, Hq * Dh), _BF16),
            pltpu.VMEM((D, Hq * Dh), _BF16),
            pltpu.VMEM((D, F), _BF16),
            pltpu.VMEM((D, F), _BF16),
            pltpu.VMEM((D, F), _BF16),
            pltpu.VMEM((4, HG, W, Dh), _BF16),
            pltpu.VMEM(((B + 1) * Hq, Dh), _F32),
            pltpu.VMEM(((B + 1) * Hq, Dh), _F32),
            pltpu.VMEM((2, B, D), _F32),
            pltpu.VMEM((B, D), A_x.dtype),
            pltpu.SemaphoreType.DMA((4,)),
            pltpu.SemaphoreType.DMA((5,)),
            pltpu.SemaphoreType.DMA((4,)),
            pltpu.SemaphoreType.DMA((3, len(DBLK) - 1)),
        ],
        compiler_params=pltpu.CompilerParams(
            vmem_limit_bytes=100 * 1024 * 1024, disable_semaphore_checks=True),
    )(A_x.reshape(B, D), A_k_cache.reshape(B * Hkv, Sk, Dh),
      A_v_cache.reshape(B * Hkv, Sk, Dh), A_wq, A_wo.T, B_w_r, B_w_gate,
      B_w_up, B_w_down.T, c, w_mod)
    return out.reshape(B, Sq, D)
```

```python
import math

import jax
import jax.numpy as jnp
from jax import lax
import jax.experimental.pallas as pl
import jax.experimental.pallas.tpu as pltpu

_NT = (((1,), (1,)), ((), ()))
_NN = (((1,), (0,)), ((), ()))
_F32 = jnp.float32
_BF16 = jnp.bfloat16
HI, LO = 0, 1


def _layernorm(x, eps=1e-05):
    m = jnp.mean(x, axis=-1, keepdims=True)
    xc = x - m
    v = jnp.mean(xc * xc, axis=-1, keepdims=True)
    return xc / jnp.sqrt(v + eps)


def _sigmoid(x):
    return 1.0 / (1.0 + jnp.exp(-x))


def _dot(a, b, dims):
    return lax.dot_general(a, b, dims, preferred_element_type=_F32)


@jax.jit
def pallas_adaLN_cond__sliding_block_cached__moe_arch_mod__decode_kernel(
    A_x: jax.Array,
    A_k_cache: jax.Array,
    A_v_cache: jax.Array,
    A_wq: jax.Array,
    A_wo: jax.Array,
    B_x: jax.Array,
    B_w_r: jax.Array,
    B_w_gate: jax.Array,
    B_w_up: jax.Array,
    B_w_down: jax.Array,
    c: jax.Array,
    w_mod: jax.Array,
):
    B, Sq, D = A_x.shape
    _, Hkv, Sk, Dh = A_k_cache.shape
    Hq = A_wq.shape[1] // Dh
    F = B_w_gate.shape[1]
    W = min(4096, max(256, Sk // 4))
    rep = Hq // Hkv
    assert (B, Sq, D, Hq, Hkv, Dh, F, W) == (8, 1, 576, 32, 16, 128, 4608, 2048)
    scale = float(Dh) ** -0.5

    HG = 8
    NG = B * Hkv // HG
    QROWS = rep * HG
    KVA = 16
    NJ = W // 128 - 1
    NF = NJ * HG
    VOFF = 3
    NSL = D // 8
    LAG = 48
    KLAG = 76
    RF = 15
    NINT = 3 * HG
    FH = F // 2
    DBLK = (0, 16, 32, 48, 64, 72)
    LB = 3
    LCH = (8, 6, 4)
    D_HI = ((0, 2), (2, 2), (4, 1))
    D_LO = ((0, 2), (2, 1), (4, 1))
    D_ORDER = 'L0 L1 R0 R1 L2 L3 L4 R2 R4 C0 C1 C2'.split()
    assert sum(LCH) * 128 == FH and KLAG + NINT <= NF

    def kernel(x_hbm, k_hbm, v_hbm, wq_hbm, wot_hbm, wr_hbm, wg_hbm, wu_hbm,
               wdt_hbm, c_hbm, wmod_hbm, out_hbm,
               xbuf, cbuf, wrbuf, wmodbuf, wqbuf, wotbuf, wgbuf, wubuf, wdtbuf,
               kvbuf, qs, os_, ep, obuf,
               misc_sems, w_sems, kv_sems, d_sems):
        cp_x = pltpu.make_async_copy(x_hbm, xbuf, misc_sems.at[0])
        cp_c = pltpu.make_async_copy(c_hbm, cbuf, misc_sems.at[1])
        cp_wr = pltpu.make_async_copy(wr_hbm, wrbuf, misc_sems.at[2])
        cp_out = pltpu.make_async_copy(obuf, out_hbm, misc_sems.at[3])

        weights = {
            'mod': (wmod_hbm, wmodbuf, 0, None, 4),
            'q': (wq_hbm, wqbuf, 1, 2, 4),
            'o': (wot_hbm, wotbuf, 2, 2, 4),
            'g': (wg_hbm, wgbuf, 3, 8, 3),
            'u': (wu_hbm, wubuf, 4, 8, 3),
        }

        def w_segs(name, prio):
            hbm, buf, s, phi, ns = weights[name]
            nt = buf.shape[1] // 128

            def rect(slab, c0, c1):
                rows = pl.ds(pl.multiple_of(slab * 8, 8), 8)
                cols = pl.ds(c0 * 128, (c1 - c0) * 128)
                pltpu.make_async_copy(hbm.at[rows, cols], buf.at[rows, cols],
                                      w_sems.at[s]).start(priority=prio)

            if phi is None:
                c0, c1 = (0, nt // 2) if prio == HI else (nt // 2, nt)
                return [(lambda i: rect((i % ns) * (NSL // ns) + i // ns, c0, c1), NSL)]
            cyc = 16 // math.gcd(nt, 16)
            ln = NSL // cyc // (2 * ns)
            segs = []
            for cc in range(ln):
                for p in range(cyc * nt // 16):
                    s0, c0 = divmod(phi + 16 * p, nt)
                    parts = [(s0, c0, min(c0 + 16, nt))]
                    if c0 + 16 > nt:
                        parts.append((s0 + 1, 0, c0 + 16 - nt))

                    def start(i, cc=cc, parts=parts):
                        k = (i + (0 if prio == HI else ns)) * ln + cc
                        for ds, c0, c1 in parts:
                            slab = k * cyc + ds
                            if prio == LO and cc == ln - 1 and ds == cyc:
                                slab = jnp.where(slab == NSL, 0, slab)
                            rect(slab, c0, c1)
                    segs.append((start, ns))
            return segs

        def w_wait(name):
            _, buf, s, _, _ = weights[name]
            pltpu.make_async_copy(buf, buf, w_sems.at[s]).wait()

        def d_rows_seg(prio, b0, nb):
            def start(i):
                blk = b0 + i % nb if nb > 1 else b0
                rows = pl.ds(pl.multiple_of((blk * 16 + i // nb) * 8, 8), 8)
                cols = pl.ds(0 if prio == HI else FH, FH)
                pltpu.make_async_copy(wdt_hbm.at[rows, cols], wdtbuf.at[rows, cols],
                                      d_sems.at[prio, blk]).start(priority=prio)
            return start, DBLK[b0 + nb] - DBLK[b0]

        def d_cols_seg(k):
            c0 = FH + sum(LCH[:k]) * 128

            def start(i):
                rows = pl.ds(pl.multiple_of(LB * 128 + (i % 2) * 64, 64), 64)
                cols = pl.ds(pl.multiple_of(c0 + (i // 2) * 256, 128), 256)
                pltpu.make_async_copy(wdt_hbm.at[rows, cols], wdtbuf.at[rows, cols],
                                      d_sems.at[2, k]).start(priority=LO)
            return start, LCH[k]

        def d_unit(name):
            kind, n = name[0], int(name[1])
            if kind == 'C':
                c0 = FH + sum(LCH[:n]) * 128
                return (LB * 128, LB * 128 + 128), (c0, c0 + LCH[n] * 128), d_sems.at[2, n]
            rows = (DBLK[n] * 8, DBLK[n + 1] * 8)
            if kind == 'L':
                return rows, (0, FH), d_sems.at[HI, n]
            return rows, (FH, F), d_sems.at[LO, n]

        def issue_loop(lo, hi, step):
            def body(i, carry):
                step(i)
                return carry
            lax.fori_loop(lo, hi, body, 0)

        def kslot(g):
            return g % 2

        def vslot(g):
            return 2 + g % 2

        def kv_pair(g, h0, nh, rk, rv, n):
            for hbm, slot, r, prio in ((v_hbm, vslot(g), rv, LO), (k_hbm, kslot(g), rk, HI)):
                pltpu.make_async_copy(
                    hbm.at[pl.ds(g * HG + h0, nh), pl.ds(Sk - W + r, n), :],
                    kvbuf.at[slot, pl.ds(h0, nh), pl.ds(r, n), :],
                    kv_sems.at[slot]).start(priority=prio)

        def kv_step(g):
            def step(u):
                j = u // HG
                jv = jnp.where(j + VOFF >= NJ, j + VOFF - NJ, j + VOFF)
                kv_pair(g, u % HG, 1, pl.multiple_of(KVA + j * 128, 16),
                        pl.multiple_of(KVA + jv * 128, 16), 128)
            return step

        def kv_edges(g):
            r = KVA + NJ * 128
            kv_pair(g, 0, HG, 0, 0, KVA)
            issue_loop(0, HG, lambda h: kv_pair(g, h, 1, r, r, W - r))

        def kv_wait(slot):
            pltpu.make_async_copy(kvbuf.at[slot], kvbuf.at[slot], kv_sems.at[slot]).wait()

        def make_issuer(lo_segs, hi_segs):
            total = max(sum(n for _, n in lo_segs), sum(n for _, n in hi_segs))
            done = [0]

            def locate(segs, pos):
                for fn, n in segs:
                    if pos < n:
                        return fn, pos, n - pos
                    pos -= n
                return None, 0, total

            def issue_to(target):
                while done[0] < min(target, total):
                    lf, li, ln = locate(lo_segs, done[0])
                    hf, hi, hn = locate(hi_segs, done[0])
                    m = min(min(target, total) - done[0], ln, hn)

                    def step(i):
                        if lf is not None:
                            lf(li + i)
                        if hf is not None:
                            hf(hi + i)
                    issue_loop(0, m, step)
                    done[0] += m
            return issue_to, total

        cp_c.start()
        cp_x.start()
        cp_wr.start()
        issue_to, n_pre = make_issuer(w_segs('mod', LO) + w_segs('q', LO) + w_segs('o', LO),
                                      w_segs('mod', HI) + w_segs('q', HI) + w_segs('o', HI))
        issue_to(n_pre // 3 + LAG)
        cp_c.wait()
        cp_x.wait()
        cf = cbuf[...].astype(_F32)
        sc = (cf * _sigmoid(cf)).astype(_BF16)
        xf = xbuf[...].astype(_F32)
        xn = _layernorm(xf)
        w_wait('mod')
        mod = _dot(sc, wmodbuf[...], _NN)
        sa, ca, ga, sb, cb, gb = [mod[:, i * D:(i + 1) * D] for i in range(6)]
        h1 = (xn * (1.0 + ca) + sa).astype(_BF16)
        issue_to(2 * n_pre // 3 + LAG)
        w_wait('q')
        q = _dot(h1, wqbuf[...], _NN)
        for hq in range(Hq):
            qs[pl.ds(hq, B, stride=Hq), :] = q[:, hq * Dh:(hq + 1) * Dh]
        issue_to(n_pre)
        kv_edges(0)
        issue_loop(0, NF, kv_step(0))

        qrow = lax.broadcasted_iota(jnp.int32, (QROWS, Dh), 0) // rep

        def attend(g, step, mid):
            ks, vs = kslot(g), vslot(g)
            rows = pl.ds(pl.multiple_of(g * QROWS, QROWS), QROWS)
            kv_wait(ks)
            kv_wait(vs)
            q16 = qs[rows, :]
            half = W // 2
            s_h = [None, None]
            for j in range(HG):
                qj = jnp.where(qrow == j, q16, 0.0).astype(_BF16)
                for hh in range(2):
                    sj = _dot(qj, kvbuf[ks, j, pl.ds(hh * half, half), :], _NT)
                    s_h[hh] = sj if s_h[hh] is None else sj + s_h[hh]
                    step(2 * j + hh)
            s = jnp.concatenate(s_h, axis=1) * scale
            m = jnp.max(s, axis=-1, keepdims=True)
            p = jnp.exp(s - m)
            l = jnp.sum(p, axis=-1, keepdims=True)
            pb = p.astype(_BF16)
            mid()
            o = jnp.zeros((QROWS, Dh), _F32)
            for j in range(HG):
                o = jnp.where(qrow == j, _dot(pb, kvbuf[vs, j], _NN), o)
                step(2 * HG + j)
            os_[rows, :] = o / l

        def period(t, carry):
            step = kv_step(t)
            kv_edges(t)
            issue_loop(0, KLAG, step)
            attend(t - 1, lambda k: step(KLAG + k), lambda: None)
            issue_loop(KLAG + NINT, NF, step)
            return carry

        lax.fori_loop(1, NG, period, 0)

        n_gu = sum(n for _, n in w_segs('g', HI))
        issue_to, n_post = make_issuer(
            w_segs('g', LO) + w_segs('u', LO) + [d_rows_seg(LO, *a) for a in D_LO]
            + [d_cols_seg(k) for k in range(len(LCH))],
            w_segs('g', HI) + w_segs('u', HI) + [d_rows_seg(HI, *a) for a in D_HI])
        issue_to(LAG)
        attend(NG - 1, lambda k: issue_to(LAG + RF) if k == HG - 1 else None,
               lambda: issue_to(LAG + 2 * RF))
        issue_to(LAG + 3 * RF)

        w_wait('o')
        cp_wr.wait()
        o_all = jnp.concatenate(
            [os_[pl.ds(hq, B, stride=Hq), :] for hq in range(Hq)], axis=1).astype(_BF16)
        hw = Hq * Dh // 2
        attn = _dot(o_all[:, :hw], wotbuf[:, pl.ds(0, hw)], _NT)
        issue_to(LAG + 4 * RF)
        attn = _dot(o_all[:, hw:], wotbuf[:, pl.ds(hw, hw)], _NT) + attn
        issue_to(LAG + 5 * RF)
        x1 = xf + ga * attn
        h2 = _layernorm(x1) * (1.0 + cb) + sb
        h2b = h2.astype(_BF16)
        wr = wrbuf[...].astype(_F32).reshape(1, D)
        r_sel = _sigmoid(jnp.sum(h2b.astype(_F32) * wr, axis=-1, keepdims=True))
        ep[0] = x1 + gb * (h2 + h2 * 0.0)
        ep[1] = gb * r_sel

        issue_to(n_gu + LAG)
        w_wait('g')
        g = _dot(h2b, wgbuf[...], _NN)
        sg = g * _sigmoid(g)
        issue_to(2 * n_gu + LAG)
        w_wait('u')
        act = (sg * _dot(h2b, wubuf[...], _NN)).astype(_BF16)
        issue_to(n_post)
        for n, name in enumerate(D_ORDER):
            (r0, r1), (c0, c1), sem = d_unit(name)
            rows, cols = pl.ds(r0, r1 - r0), pl.ds(c0, c1 - c0)
            pltpu.make_async_copy(wdtbuf.at[rows, cols], wdtbuf.at[rows, cols], sem).wait()
            y = _dot(act[:, c0:c1], wdtbuf[rows, cols], _NT)
            acc = ep[0, :, rows] + ep[1, :, rows] * y
            if any(d_unit(later)[0] == (r0, r1) for later in D_ORDER[n + 1:]):
                ep[0, :, rows] = acc
            else:
                obuf[:, rows] = acc.astype(obuf.dtype)
        cp_out.start()
        cp_out.wait()

    any_spec = pl.BlockSpec(memory_space=pl.ANY)
    out = pl.pallas_call(
        kernel,
        out_shape=jax.ShapeDtypeStruct((B, D), A_x.dtype),
        in_specs=[any_spec] * 11,
        out_specs=any_spec,
        scratch_shapes=[
            pltpu.VMEM((B, D), _BF16),
            pltpu.VMEM((B, D), _BF16),
            pltpu.VMEM((D,), _BF16),
            pltpu.VMEM((D, 6 * D), _BF16),
            pltpu.VMEM((D, Hq * Dh), _BF16),
            pltpu.VMEM((D, Hq * Dh), _BF16),
            pltpu.VMEM((D, F), _BF16),
            pltpu.VMEM((D, F), _BF16),
            pltpu.VMEM((D, F), _BF16),
            pltpu.VMEM((4, HG, W, Dh), _BF16),
            pltpu.VMEM(((B + 1) * Hq, Dh), _F32),
            pltpu.VMEM(((B + 1) * Hq, Dh), _F32),
            pltpu.VMEM((2, B, D), _F32),
            pltpu.VMEM((B, D), A_x.dtype),
            pltpu.SemaphoreType.DMA((4,)),
            pltpu.SemaphoreType.DMA((5,)),
            pltpu.SemaphoreType.DMA((4,)),
            pltpu.SemaphoreType.DMA((3, len(DBLK) - 1)),
        ],
        compiler_params=pltpu.CompilerParams(
            vmem_limit_bytes=100 * 1024 * 1024, disable_semaphore_checks=True),
    )(A_x.reshape(B, D), A_k_cache.reshape(B * Hkv, Sk, Dh),
      A_v_cache.reshape(B * Hkv, Sk, Dh), A_wq, A_wo.T, B_w_r, B_w_gate,
      B_w_up, B_w_down.T, c, w_mod)
    return out.reshape(B, Sq, D)
```
